```python
import os as _os
_os.environ.setdefault("JAX_PLATFORMS", "cpu")
import jax
import jax.numpy as jnp

def _softmax(x, axis=-1):
    return jax.nn.softmax(x, axis=axis)
def _gelu(x):
    return jax.nn.gelu(x, approximate=True)
def _silu(x):
    return jax.nn.silu(x)
def _sigmoid(x):
    return jax.nn.sigmoid(x)
def _layernorm(x, axis=-1, eps=1e-5):
    m = jnp.mean(x, axis=axis, keepdims=True)
    v = jnp.var(x, axis=axis, keepdims=True)
    return (x - m) / jnp.sqrt(v + eps)
def _scatter_add(tgt, idx, src, axis=0):
    return tgt.at[idx].add(src)
def _segment_sum(src, seg, n):
    return jax.ops.segment_sum(src, seg, n)
class _Rng:
    def __init__(self, key):
        self._k = key
    def _next(self):
        self._k, sub = jax.random.split(self._k)
        return sub
    def normal(self, shape):
        return jax.random.normal(self._next(), shape, dtype=jnp.bfloat16)
    def randint(self, lo, hi, shape):
        return jax.random.randint(self._next(), shape, lo, hi, dtype=jnp.int32)
    def uniform(self, shape, lo=0.0, hi=1.0):
        return jax.random.uniform(self._next(), shape, jnp.bfloat16, lo, hi)
    def permutation(self, n):
        return jax.random.permutation(self._next(), n)


kernel_name = 'standalone__fft_conv__vision'

def setup_inputs():
    _rng = _Rng(jax.random.key(int.from_bytes(__import__("os").urandom(4), "little")))
    _w = (lambda a: (lambda t: t.astype(jnp.bfloat16) if jnp.issubdtype(t.dtype, jnp.floating) else t)(jnp.asarray(a)))
    H = W = 224
    C = 96
    K = 3
    return {
        "x": _w((lambda *s: _rng.normal(s) * 0.05)(1, H, W, C)),
        "w": _w((lambda *s: _rng.normal(s) * 0.05)(K, K, C, C)),
    }

def reference(x, w):
    B, H, W, C = x.shape
    K = w.shape[0]
    wp = jnp.pad(w, ((0, H - K), (0, W - K), (0, 0), (0, 0)))
    Xf = (lambda x, axes=(-2,-1): jnp.fft.rfft2(x.astype(jnp.float32), axes=axes))(x, axes=(1, 2))
    Wf = (lambda x, axes=(-2,-1): jnp.fft.rfft2(x.astype(jnp.float32), axes=axes))(wp, axes=(0, 1))
    Yf = jnp.einsum('bhwi,hwio->bhwo', Xf, Wf)
    y = (lambda x, s, axes=(-2,-1): jnp.fft.irfft2(x, s=s, axes=axes).astype(jnp.bfloat16))(Yf, (H, W), axes=(1, 2))
    return y
```

```python
import numpy as np
import jax
import jax.numpy as jnp
import jax.experimental.pallas as pl
import jax.experimental.pallas.tpu as pltpu

_BF16 = jnp.bfloat16
_F32 = jnp.float32

_IN_CHUNKS = (8, 16, 32, 56, 56, 56)
_OUT_CHUNKS = (32,) * 6 + (16, 8, 4, 4)
_OUT_DELAY = 64


def _make_kernel(H, W, C):
    assert H == 224 and W == 224 and C == 96
    in_chunks, out_chunks = _IN_CHUNKS, _OUT_CHUNKS
    in_starts = np.concatenate([[0], np.cumsum(in_chunks)]).tolist()
    out_starts = np.concatenate([[0], np.cumsum(out_chunks)]).tolist()
    NI, NO, NG = len(in_chunks), len(out_chunks), H // 4

    def kernel(x_hbm, w_hbm, o_hbm, xs, ys, wv, in_sems, out_sem):
        def in_copy(i):
            s, n = in_starts[i], in_chunks[i]
            return pltpu.make_async_copy(
                x_hbm.at[pl.ds(s, n)], xs.at[pl.ds(2 + s, n)], in_sems.at[i])

        def out_copy(i):
            s, n = out_starts[i], out_chunks[i]
            return pltpu.make_async_copy(
                ys.at[pl.ds(s, n)], o_hbm.at[pl.ds(s, n)], out_sem)

        wcp = pltpu.make_async_copy(w_hbm, wv, in_sems.at[NI + 1])
        wcp.start()
        halo = pltpu.make_async_copy(
            x_hbm.at[pl.ds(H - 2, 2)], xs.at[pl.ds(0, 2)], in_sems.at[NI])
        halo.start()
        for i in range(NI):
            in_copy(i).start()
        wcp.wait()

        def packrows(a):
            return [pltpu.pack_elementwise(
                [a[16 * j:16 * j + 8], a[16 * j + 8:16 * j + 16]], packed_dtype=_BF16)
                for j in range(a.shape[0] // 16)]

        gt = [[] for _ in range(6)]
        rt = []
        for kw in range(3):
            g0 = wv[2, kw].astype(_F32)
            g1 = wv[1, kw].astype(_F32)
            g2 = wv[0, kw].astype(_F32)
            if kw == 2:
                rt = packrows(g0[64:]) + packrows(g1[64:]) + packrows(g2[64:])
                g0, g1, g2 = g0[:64], g1[:64], g2[:64]
            e = g0 + g2
            e2 = g0 * (1 / 24) + g2 * (1 / 6)
            o2 = g1 * (1 / 12)
            for i, gi in enumerate([g0 * 0.25, (e + g1) * (-1 / 6), (e - g1) * (-1 / 6),
                                    e2 + o2, e2 - o2, g2]):
                gt[i] += packrows(gi)
        eye = (jax.lax.broadcasted_iota(jnp.int32, (C, C), 0)
               == jax.lax.broadcasted_iota(jnp.int32, (C, C), 1)).astype(_BF16)

        def transpose(lst):
            a = pltpu.bitcast(jnp.concatenate(lst, axis=0), _BF16)
            return jax.lax.dot_general(
                eye, a, (((1,), (1,)), ((), ())), preferred_element_type=_F32).astype(_BF16)

        gm = [transpose(gt[i]) for i in range(6)]
        gr = transpose(rt)
        g0r = jnp.concatenate([gm[0], gr], axis=1)
        g5r = jnp.concatenate([gm[5], gr], axis=1)
        halo.wait()

        lane = jax.lax.broadcasted_iota(jnp.int32, (8, 128), 1)

        def pack2(lo, hi):
            p = pltpu.pack_elementwise([lo, hi], packed_dtype=_BF16)
            v0 = p[:, :128]
            u = jnp.concatenate([p[:, 128:], v0[:, 96:]], axis=1)
            return v0, u

        def shifted(v0, u, k):
            o0 = jnp.where(lane < k, pltpu.roll(u, 32 + k, 1), pltpu.roll(v0, k, 1))
            o1 = pltpu.roll(u, k, 1)
            return jnp.concatenate([o0, o1], axis=1)

        def btrans(d):
            a_ = d[4] - 4.0 * d[2]
            b_ = d[3] - 4.0 * d[1]
            c_ = d[4] - d[2]
            f_ = d[3] - d[1]
            e_ = f_ + f_
            return [4.0 * (d[0] - d[2]) + c_, a_ + b_, a_ - b_, c_ + e_, c_ - e_,
                    (d[5] - d[3]) - (e_ + e_)]

        rr = {}

        def build(q):
            b = 4 * q
            p0 = [[] for _ in range(6)]
            p1 = [[] for _ in range(6)]
            p2 = [[] for _ in range(6)]
            newr = [r for r in range(b, b + 6) if r not in rr]
            for r in newr:
                rr[r] = []
            for j in range(6):
                dl = [xs[b + k, 16 * j:16 * j + 8, :].astype(_F32) for k in range(6)]
                dh = [xs[b + k, 16 * j + 8:16 * j + 16, :].astype(_F32) for k in range(6)]
                tl, th = btrans(dl), btrans(dh)
                for i in range(6):
                    v0, u = pack2(tl[i], th[i])
                    p0[i].append(jnp.concatenate([v0, u], axis=1))
                    p1[i].append(shifted(v0, u, 1))
                    if j < 4:
                        p2[i].append(shifted(v0, u, 2))
                if j >= 4:
                    for r in newr:
                        rr[r].append(shifted(*pack2(dl[r - b], dh[r - b]), 2))
            t = [pltpu.bitcast(jnp.concatenate(p0[i] + p1[i] + p2[i], axis=0), _BF16)
                 for i in range(6)]
            r_ = [pltpu.bitcast(jnp.concatenate(rr[b + j] + rr[b + j + 1] + rr[b + j + 2],
                                                axis=0), _BF16) for j in range(4)]
            for r in range(b, b + 4):
                del rr[r]
            return t, r_

        def dot(g, x):
            return jnp.dot(g, x, preferred_element_type=_F32)

        st = dict(waited=0, nout=0)

        def wait_for(q):
            while in_starts[st['waited']] < 4 * q + 4:
                in_copy(st['waited']).wait()
                st['waited'] += 1

        def compute(q, t, r_):
            b = 4 * q
            m1 = dot(gm[1], t[1])
            m2 = dot(gm[2], t[2])
            m3 = dot(gm[3], t[3])
            m4 = dot(gm[4], t[4])
            m0 = dot(g0r, jnp.concatenate([t[0], r_[0]], axis=0))
            r1 = dot(gr, r_[1])
            r2 = dot(gr, r_[2])
            m5 = dot(g5r, jnp.concatenate([t[5], r_[3]], axis=0))
            s1, d1, s2, d2 = m1 + m2, m1 - m2, m3 + m4, m3 - m4
            y = [m0 + s1 + s2, d1 + 2.0 * d2 + r1, s1 + 4.0 * s2 + r2, d1 + 8.0 * d2 + m5]
            for j in range(4):
                ys[b + j] = y[j][:, :W].astype(_BF16)
            if b + 4 >= _OUT_DELAY:
                while st['nout'] < NO and out_starts[st['nout'] + 1] <= b + 4:
                    out_copy(st['nout']).start()
                    st['nout'] += 1

        wait_for(0)
        cur = build(0)
        for q in range(NG):
            nxt = None
            if q + 1 < NG:
                wait_for(q + 1)
                nxt = build(q + 1)
            compute(q, *cur)
            cur = nxt
        for i in range(NO):
            out_copy(i).wait()

    return kernel, NI


@jax.jit
def pallas_standalone__fft_conv__vision_kernel(x: jax.Array, w: jax.Array):
    _, H, W, C = x.shape
    kernel, ni = _make_kernel(H, W, C)
    xt = jnp.transpose(x[0], (0, 2, 1))
    yt = pl.pallas_call(
        kernel,
        in_specs=[pl.BlockSpec(memory_space=pl.ANY), pl.BlockSpec(memory_space=pl.ANY)],
        out_specs=pl.BlockSpec(memory_space=pl.ANY),
        out_shape=jax.ShapeDtypeStruct((H, C, W), _BF16),
        scratch_shapes=[
            pltpu.VMEM((H + 2, C, W), _BF16),
            pltpu.VMEM((H, C, W), _BF16),
            pltpu.VMEM((3, 3, C, C), _BF16),
            pltpu.SemaphoreType.DMA((ni + 2,)),
            pltpu.SemaphoreType.DMA(()),
        ],
        compiler_params=pltpu.CompilerParams(
            vmem_limit_bytes=100 * 2**20,
            disable_bounds_checks=True,
            disable_semaphore_checks=True,
        ),
    )(xt, w)
    return jnp.transpose(yt, (0, 2, 1))[None]
```

```python
import numpy as np
import jax
import jax.numpy as jnp
import jax.experimental.pallas as pl
import jax.experimental.pallas.tpu as pltpu

_BF16 = jnp.bfloat16
_F32 = jnp.float32

_SIZES = (4,) + (6,) * 36 + (4,)
_IN_BOUNDS = (4, 10, 22, 46, 88, 160)
_PATTERN = "0 r1' r2' 7 r3' r4' 1 2 3 4 5 6"
_LEAD = 1
_W_START, _W_RATE, _W_MARGIN = 102, 1.85, 12
_COEF = {
    4: [(1, 1), (1, 2), (1, 4), (1, 8)],
    6: [(1, 1, 1), (1, 2, .5), (1, 4, .25), (1, 8, .125), (1, 16, .0625), (1, 32, .03125)],
}


def _tr4(d):
    a = d[4] - 4.0 * d[2]
    b = d[3] - 4.0 * d[1]
    c = a + 3.0 * d[2]
    f = b + 3.0 * d[1]
    e = f + f
    return {0: d[0] + 0.25 * (a - d[2]), 1: 0.75 * (a + b), 2: 0.75 * (a - b),
            3: 3.75 * (c + e), 4: 3.75 * (c - e), 7: (d[5] - 4.0 * d[3]) - b}


def _tr6(d):
    p = d[4] - d[2]
    e3 = (d[6] - d[4]) - 4.0 * p
    t0 = ((d[0] - d[2]) + 0.25 * p) - e3
    s = d[5] - d[3]
    h = 4.0 * s - (d[3] - d[1])
    t7 = ((d[7] - d[5]) - 0.25 * s) - h
    e2 = e3 + 3.75 * p
    e1 = (e3 + 3.0 * p) - 2.25 * d[4]
    o2 = 0.5 * h
    o3 = 2.0 * h - 7.5 * s
    o1 = (h - 3.0 * s) - 2.25 * d[3]
    return {0: t0, 1: e1 + o1, 2: e1 - o1, 3: e2 + o2, 4: e2 - o2, 5: e3 + o3, 6: e3 - o3, 7: t7}


def _make_kernel(H, W, C):
    assert H == 224 and W == 224 and C == 96 and sum(_SIZES) == H
    sizes = _SIZES
    pat = [(-1, t[:-1]) if t.endswith("'") else (0, t) for t in _PATTERN.split()]
    gstart = np.concatenate([[0], np.cumsum(sizes)]).tolist()
    in_starts = [0] + list(_IN_BOUNDS) + [H - 2]
    NI, NG = len(in_starts) - 1, len(sizes)

    def kernel(x_hbm, w_hbm, o_hbm, xs, ys, wv, in_sems, out_sem):
        def in_copy(i):
            s, n = in_starts[i], in_starts[i + 1] - in_starts[i]
            return pltpu.make_async_copy(
                x_hbm.at[pl.ds(s, n)], xs.at[pl.ds(s, n)], in_sems.at[i])

        wcp = pltpu.make_async_copy(w_hbm, wv, in_sems.at[NI + 1])
        wcp.start()
        halo = pltpu.make_async_copy(
            x_hbm.at[pl.ds(H - 2, 2)], xs.at[pl.ds(H - 2, 2)], in_sems.at[NI])
        halo.start()
        for i in range(NI):
            in_copy(i).start()
        wcp.wait()

        def packrows(a):
            return [pltpu.pack_elementwise(
                [a[16 * j:16 * j + 8], a[16 * j + 8:16 * j + 16]], packed_dtype=_BF16)
                for j in range(a.shape[0] // 16)]

        eye = (jax.lax.broadcasted_iota(jnp.int32, (C, C), 0)
               == jax.lax.broadcasted_iota(jnp.int32, (C, C), 1)).astype(_BF16)

        def transpose(lst):
            a = pltpu.bitcast(jnp.concatenate(lst, axis=0), _BF16)
            return jax.lax.dot_general(
                eye, a, (((1,), (1,)), ((), ())), preferred_element_type=_F32)

        pw = [[packrows(wv[2 - k, kw].astype(_F32)) for kw in range(3)] for k in range(3)]
        gr = transpose(pw[0][2][4:] + pw[1][2][4:] + pw[2][2][4:]).astype(_BF16)
        g0, g1, g2 = [transpose(pw[k][0] + pw[k][1] + pw[k][2][:4]) for k in range(3)]
        e1, o1 = (g0 + g2) * (-2 / 9), g1 * (-2 / 9)
        e2, o2 = g0 * (1 / 90) + g2 * (2 / 45), g1 * (1 / 45)
        e3, o3 = g0 * (32 / 45) + g2 * (8 / 45), g1 * (16 / 45)
        gm = [g.astype(_BF16) for g in
              [g0, e1 + o1, e1 - o1, e2 + o2, e2 - o2, e3 + o3, e3 - o3, g2]]
        g0r = jnp.concatenate([gm[0], gr], axis=1)
        g7r = jnp.concatenate([gm[7], gr], axis=1)
        halo.wait()
        in_copy(0).wait()

        lane = jax.lax.broadcasted_iota(jnp.int32, (8, 128), 1)

        def pack2(lo, hi):
            p = pltpu.pack_elementwise([lo, hi], packed_dtype=_BF16)
            v0 = p[:, :128]
            u = jnp.concatenate([p[:, 128:], v0[:, 96:]], axis=1)
            return v0, u

        def shifted(v0, u, k):
            o0 = jnp.where(lane < k, pltpu.roll(u, 32 + k, 1), pltpu.roll(v0, k, 1))
            o1 = pltpu.roll(u, k, 1)
            return jnp.concatenate([o0, o1], axis=1)

        rr = {}

        def build(g):
            b, m = gstart[g], sizes[g]
            n = m + 2
            tr = _tr6 if m == 6 else _tr4
            keys = [0, 1, 2, 3, 4, 5, 6, 7] if m == 6 else [0, 1, 2, 3, 4, 7]
            p0 = {i: [] for i in keys}
            p1 = {i: [] for i in keys}
            p2 = {i: [] for i in keys}
            newr = [r for r in range(b, b + n) if r not in rr]
            for r in newr:
                rr[r] = []
            for j in range(6):
                dl = [xs[(b + k - 2) % H, 16 * j:16 * j + 8, :].astype(_F32) for k in range(n)]
                dh = [xs[(b + k - 2) % H, 16 * j + 8:16 * j + 16, :].astype(_F32)
                      for k in range(n)]
                tl, th = tr(dl), tr(dh)
                for i in keys:
                    v0, u = pack2(tl[i], th[i])
                    p0[i].append(jnp.concatenate([v0, u], axis=1))
                    p1[i].append(shifted(v0, u, 1))
                    if j < 4:
                        p2[i].append(shifted(v0, u, 2))
                if j >= 4:
                    for r in newr:
                        rr[r].append(shifted(*pack2(dl[r - b], dh[r - b]), 2))
            t = {i: pltpu.bitcast(jnp.concatenate(p0[i] + p1[i] + p2[i], axis=0), _BF16)
                 for i in keys}
            r_ = [pltpu.bitcast(jnp.concatenate(rr[b + j] + rr[b + j + 1] + rr[b + j + 2],
                                                axis=0), _BF16) for j in range(m)]
            for r in range(b, b + m):
                del rr[r]
            return t, r_

        def dot(g, x):
            return jnp.dot(g, x, preferred_element_type=_F32)

        def product(t, r_, tok):
            if tok == '0':
                return dot(g0r, jnp.concatenate([t[0], r_[0]], axis=0))
            if tok == '7':
                return dot(g7r, jnp.concatenate([t[7], r_[-1]], axis=0))
            if tok[0] == 'r':
                return dot(gr, r_[int(tok[1:])])
            return dot(gm[int(tok)], t[int(tok)])

        st = dict(waited=1)
        built, prods, sd = {}, {g: {} for g in range(NG)}, {}
        done, written = set(), set()

        def wait_for(g):
            while st['waited'] < NI and in_starts[st['waited']] < gstart[g + 1]:
                in_copy(st['waited']).wait()
                st['waited'] += 1

        def pair(g, k, odd):
            if (g, k, odd) not in sd:
                a, b = prods[g][str(2 * k + 1)], prods[g][str(2 * k + 2)]
                sd[g, k, odd] = a - b if odd else a + b
            return sd[g, k, odd]

        def finalize(g):
            m, ms = sizes[g], prods[g]
            if not all(str(i) in ms for i in range(1, m + 1)):
                return
            for j in range(m):
                key = '0' if j == 0 else ('7' if j == m - 1 else 'r%d' % j)
                row = gstart[g] + j
                if row in done or key not in ms:
                    continue
                terms = [pair(g, k, j % 2) if c == 1 else c * pair(g, k, j % 2)
                         for k, c in enumerate(_COEF[m][j])]
                terms = [ms[key]] + terms if j == 0 else terms + [ms[key]]
                y = terms[0]
                for term in terms[1:]:
                    y = y + term
                ys[row] = y[:, :W].astype(_BF16)
                done.add(row)
            avail = sorted(done - written)
            if len(done) < _W_START or not avail:
                return
            target = H if len(done) == H else int((len(done) - _W_START) * _W_RATE + _W_MARGIN)
            k = min(target - len(written), len(avail))
            if k <= 0:
                return
            rows = [avail[int((i + 0.5) * len(avail) / k)] for i in range(k)]
            hop = max(1, int(round(k ** 0.5)))
            for r in [rows[i] for s in range(hop) for i in range(s, k, hop)]:
                pltpu.make_async_copy(
                    ys.at[pl.ds(r, 1)], o_hbm.at[pl.ds(r, 1)], out_sem).start()
                written.add(r)

        seq = []
        for g in range(NG + 1):
            for dg, tok in pat:
                gg = g + dg
                if 0 <= gg < NG and not (sizes[gg] == 4 and tok in ('5', '6', 'r3', 'r4')):
                    seq.append((gg, tok))
        first = {}
        for pos, (g, _) in enumerate(seq):
            first.setdefault(g, pos)
        waitpos = {max(first[g] - _LEAD, first[g - 1] + 1): g for g in range(1, NG)}
        for pos, (g, tok) in enumerate(seq):
            if pos in waitpos:
                wait_for(waitpos[pos])
            if g not in built:
                built[g] = build(g)
            prods[g][tok] = product(*built[g], tok)
            finalize(g)
        assert len(written) == H and st['waited'] == NI
        pltpu.make_async_copy(ys, o_hbm, out_sem).wait()

    return kernel, NI


@jax.jit
def pallas_standalone__fft_conv__vision_kernel(x: jax.Array, w: jax.Array):
    _, H, W, C = x.shape
    kernel, ni = _make_kernel(H, W, C)
    xt = jnp.transpose(x[0], (0, 2, 1))
    yt = pl.pallas_call(
        kernel,
        in_specs=[pl.BlockSpec(memory_space=pl.ANY), pl.BlockSpec(memory_space=pl.ANY)],
        out_specs=pl.BlockSpec(memory_space=pl.ANY),
        out_shape=jax.ShapeDtypeStruct((H, C, W), _BF16),
        scratch_shapes=[
            pltpu.VMEM((H, C, W), _BF16),
            pltpu.VMEM((H, C, W), _BF16),
            pltpu.VMEM((3, 3, C, C), _BF16),
            pltpu.SemaphoreType.DMA((ni + 2,)),
            pltpu.SemaphoreType.DMA(()),
        ],
        compiler_params=pltpu.CompilerParams(
            vmem_limit_bytes=100 * 2**20,
            disable_bounds_checks=True,
            disable_semaphore_checks=True,
        ),
    )(xt, w)
    return jnp.transpose(yt, (0, 2, 1))[None]
```

```python
import numpy as np
import jax
import jax.numpy as jnp
import jax.experimental.pallas as pl
import jax.experimental.pallas.tpu as pltpu

_BF16 = jnp.bfloat16
_F32 = jnp.float32

_SIZES = (4,) + (6,) * 36 + (4,)
_IN_BOUNDS = (4, 10, 22, 40, 76, 142, 220)
_LEADS = (3, 4, 6, 6, 6, 6, 6)
_PRE = 3
_PATTERN = "0' 7 r1' r2' r3' r4' 1 2 3 4 5 6"
_PATTERN0 = "r1 r2 1 2 7 3 4"
_W_START, _W_RATE, _W_MARGIN, _W_FINE = 102, 1.75, 16, 214

_COEF = {
    4: [(1, 1), (1, 2), (1, 4), (1, 8)],
    6: [(1, 1, 1), (1, 2, .5), (1, 4, .25), (1, 8, .125), (1, 16, .0625), (1, 32, .03125)],
}
_ADD = lambda a, b: a + b
_SUB = lambda a, b: a - b
_GRAPH = {
    6: {
        'p': (_SUB, ('d4', 'd2')),
        'e3': (lambda d6, d4, p: (d6 - d4) - 4.0 * p, ('d6', 'd4', 'p')),
        't0': (lambda d0, d2, p, e3: ((d0 - d2) + 0.25 * p) - e3, ('d0', 'd2', 'p', 'e3')),
        's': (_SUB, ('d5', 'd3')),
        'h': (lambda s, d3, d1: 0.25 * s - (d3 - d1), ('s', 'd3', 'd1')),
        't7': (lambda d7, d5, s, h: ((d7 - d5) - 4.0 * s) - h, ('d7', 'd5', 's', 'h')),
        'e2': (lambda e3, p: e3 + 3.75 * p, ('e3', 'p')),
        'e1': (lambda e3, p, d4: (e3 + 3.0 * p) - 2.25 * d4, ('e3', 'p', 'd4')),
        'o3': (lambda h: h + h, ('h',)),
        'o2': (lambda h, s: 0.5 * h + 1.875 * s, ('h', 's')),
        'o1': (lambda h, s, d3: (h + 0.75 * s) - 2.25 * d3, ('h', 's', 'd3')),
        't1': (_ADD, ('e1', 'o1')), 't2': (_SUB, ('e1', 'o1')),
        't3': (_ADD, ('e2', 'o2')), 't4': (_SUB, ('e2', 'o2')),
        't5': (_ADD, ('e3', 'o3')), 't6': (_SUB, ('e3', 'o3')),
    },
    4: {
        'a': (lambda d4, d2: d4 - 4.0 * d2, ('d4', 'd2')),
        'b': (lambda d3, d1: d3 - 4.0 * d1, ('d3', 'd1')),
        'c': (lambda a, d2: a + 3.0 * d2, ('a', 'd2')),
        'f': (lambda b, d1: b + 3.0 * d1, ('b', 'd1')),
        'e': (lambda f: f + f, ('f',)),
        't0': (lambda d0, a, d2: d0 + 0.25 * (a - d2), ('d0', 'a', 'd2')),
        't1': (lambda a, b: 0.75 * (a + b), ('a', 'b')),
        't2': (lambda a, b: 0.75 * (a - b), ('a', 'b')),
        't3': (lambda c, e: 3.75 * (c + e), ('c', 'e')),
        't4': (lambda c, e: 3.75 * (c - e), ('c', 'e')),
        't7': (lambda d5, d3, b: (d5 - 4.0 * d3) - b, ('d5', 'd3', 'b')),
    },
}


def _schedule(sizes, gstart, in_starts):
    ng = len(sizes)
    seq = []
    for g in range(ng + 1):
        for tok in (_PATTERN0 if g == 0 else _PATTERN).split():
            gg, tok = (g - 1, tok[:-1]) if tok.endswith("'") else (g, tok)
            if not 0 <= gg < ng or (gg, tok) in seq:
                continue
            if sizes[gg] == 4 and tok in ('5', '6', 'r3', 'r4'):
                continue
            seq.append((gg, tok))
    assert len(seq) == sum(2 * m for m in sizes)
    first = {}
    for pos, (g, _) in enumerate(seq):
        first.setdefault(g, pos)
    waits = {}
    for i, lead in enumerate(_LEADS, start=1):
        g = gstart.index(in_starts[i])
        waits[max(first[g] - lead, first[g - 1] + 1)] = (i, g)
    return seq, waits


def _make_kernel(H, W, C):
    assert H == 224 and W == 224 and C == 96 and sum(_SIZES) == H
    sizes = _SIZES
    gstart = np.concatenate([[0], np.cumsum(sizes)]).tolist()
    in_starts = [0] + list(_IN_BOUNDS) + [H - 2]
    NI = len(in_starts) - 1
    seq, waits = _schedule(sizes, gstart, in_starts)
    assert len(waits) == NI - 1

    def kernel(x_hbm, w_hbm, o_hbm, xs, ys, wv, in_sems, out_sem):
        def in_copy(i):
            s, n = in_starts[i], in_starts[i + 1] - in_starts[i]
            return pltpu.make_async_copy(
                x_hbm.at[pl.ds(s, n)], xs.at[pl.ds(s, n)], in_sems.at[i])

        wcp = pltpu.make_async_copy(w_hbm, wv, in_sems.at[NI + 1])
        wcp.start()
        halo = pltpu.make_async_copy(
            x_hbm.at[pl.ds(H - 2, 2)], xs.at[pl.ds(H - 2, 2)], in_sems.at[NI])
        halo.start()
        for i in range(NI):
            in_copy(i).start()
        wcp.wait()

        eye = (jax.lax.broadcasted_iota(jnp.int32, (C, C), 0)
               == jax.lax.broadcasted_iota(jnp.int32, (C, C), 1)).astype(_BF16)

        def transpose(lst):
            return jax.lax.dot_general(
                eye, jnp.concatenate(lst, axis=0), (((1,), (1,)), ((), ())),
                preferred_element_type=_F32)

        pw = [[wv[2 - k, kw] for kw in range(3)] for k in range(3)]
        gr = transpose([pw[k][2][64:] for k in range(3)]).astype(_BF16)
        g0, g1, g2 = [transpose([pw[k][0], pw[k][1], pw[k][2][:64]]) for k in range(3)]
        e1, o1 = (g0 + g2) * (-2 / 9), g1 * (-2 / 9)
        e2, o2 = g0 * (1 / 90) + g2 * (2 / 45), g1 * (1 / 45)
        e3, o3 = g0 * (32 / 45) + g2 * (8 / 45), g1 * (16 / 45)
        gm = [g.astype(_BF16) for g in
              [g0, e1 + o1, e1 - o1, e2 + o2, e2 - o2, e3 + o3, e3 - o3, g2]]
        gm[0] = jnp.concatenate([gm[0], gr], axis=1)
        gm[7] = jnp.concatenate([gm[7], gr], axis=1)
        halo.wait()
        in_copy(0).wait()

        def split2(v):
            p = pltpu.bitcast(v, jnp.uint32)
            v0 = p[:, :128]
            return v0, jnp.concatenate([p[:, 128:], v0[:, 96:]], axis=1)

        def shifted(v0, u, k):
            lane = jax.lax.broadcasted_iota(jnp.int32, v0.shape, 1)
            o0 = jnp.where(lane < k, pltpu.roll(u, 32 + k, 1), pltpu.roll(v0, k, 1))
            return jnp.concatenate([o0, pltpu.roll(u, k, 1)], axis=1)

        vals, rest_rows, rhss, pairs = {}, {}, {}, {}
        prods = {g: {} for g in range(len(sizes))}
        done, written = set(), set()

        def val(g, name):
            if (g, name) not in vals:
                if name[0] == 'd':
                    vals[g, name] = xs[(gstart[g] + int(name[1:]) - 2) % H].astype(_F32)
                else:
                    fn, deps = _GRAPH[sizes[g]][name]
                    vals[g, name] = fn(*[val(g, d) for d in deps])
            return vals[g, name]

        def rest(r):
            if r not in rest_rows:
                rest_rows[r] = shifted(*split2(xs[(r - 2) % H, 64:96, :]), 2)
            return rest_rows[r]

        def rhs(g, tok):
            if (g, tok) not in rhss:
                parts = []
                if tok[0] != 'r':
                    v0, u = split2(val(g, 't' + tok).astype(_BF16))
                    parts += [jnp.concatenate([v0, u], axis=1), shifted(v0, u, 1),
                              shifted(v0[:32], u[:32], 2)]
                if tok[0] == 'r' or tok in ('0', '7'):
                    j = int(tok[1:]) if tok[0] == 'r' else (0 if tok == '0' else sizes[g] - 1)
                    parts += [rest(gstart[g] + j + k) for k in range(3)]
                rhss[g, tok] = pltpu.bitcast(jnp.concatenate(parts, axis=0), _BF16)
            return rhss[g, tok]

        def pair(g, k, odd):
            if (g, k, odd) not in pairs:
                a, b = prods[g][str(2 * k + 1)], prods[g][str(2 * k + 2)]
                pairs[g, k, odd] = a - b if odd else a + b
            return pairs[g, k, odd]

        def finalize(g):
            m, ms = sizes[g], prods[g]
            if not all(str(i) in ms for i in range(1, m + 1)):
                return
            for j in range(m):
                key = '0' if j == 0 else ('7' if j == m - 1 else 'r%d' % j)
                row = gstart[g] + j
                if row in done or key not in ms:
                    continue
                terms = [pair(g, k, j % 2) if c == 1 else c * pair(g, k, j % 2)
                         for k, c in enumerate(_COEF[m][j])]
                terms = [ms[key]] + terms if j == 0 else terms + [ms[key]]
                y = terms[0]
                for term in terms[1:]:
                    y = y + term
                ys[row] = y[:, :W].astype(_BF16)
                done.add(row)
            avail, nd = sorted(done - written), len(done)
            if nd < _W_START or (nd < _W_FINE and (nd - 4) % 6 not in (0, 2)):
                return
            target = H if nd == H else int((nd - _W_START) * _W_RATE + _W_MARGIN)
            for _ in range(min(target - len(written), len(avail))):
                r = avail.pop(int((len(written) * 0.381966) % 1.0 * len(avail)))
                pltpu.make_async_copy(
                    ys.at[pl.ds(r, 1)], o_hbm.at[pl.ds(r, 1)], out_sem).start()
                written.add(r)

        for pos, (g, tok) in enumerate(seq):
            if pos in waits:
                chunk, gw = waits[pos]
                for g2, tok2 in seq[pos:pos + _PRE]:
                    if g2 < gw:
                        rhs(g2, tok2)
                in_copy(chunk).wait()
                for key in [key for key in vals if key[1][0] == 'd']:
                    del vals[key]
            lhs = gr if tok[0] == 'r' else gm[int(tok)]
            prods[g][tok] = jnp.dot(lhs, rhs(g, tok), preferred_element_type=_F32)
            finalize(g)
        assert len(written) == H
        pltpu.make_async_copy(ys, o_hbm, out_sem).wait()

    return kernel, NI


def _compiler_params():
    base = dict(vmem_limit_bytes=48 * 2**20)
    try:
        return pltpu.CompilerParams(disable_semaphore_checks=True, **base)
    except TypeError:
        return pltpu.CompilerParams(**base)


@jax.jit
def pallas_standalone__fft_conv__vision_kernel(x: jax.Array, w: jax.Array):
    _, H, W, C = x.shape
    kernel, ni = _make_kernel(H, W, C)
    xt = jnp.transpose(x[0], (0, 2, 1))
    yt = pl.pallas_call(
        kernel,
        in_specs=[pl.BlockSpec(memory_space=pl.ANY), pl.BlockSpec(memory_space=pl.ANY)],
        out_specs=pl.BlockSpec(memory_space=pl.ANY),
        out_shape=jax.ShapeDtypeStruct((H, C, W), _BF16),
        scratch_shapes=[
            pltpu.VMEM((H, C, W), _BF16),
            pltpu.VMEM((H, C, W), _BF16),
            pltpu.VMEM((3, 3, C, C), _BF16),
            pltpu.SemaphoreType.DMA((ni + 2,)),
            pltpu.SemaphoreType.DMA(()),
        ],
        compiler_params=_compiler_params(),
    )(xt, w)
    return jnp.transpose(yt, (0, 2, 1))[None]
```
